```python
import os as _os
_os.environ.setdefault("JAX_PLATFORMS", "cpu")
import jax
import jax.numpy as jnp

def _softmax(x, axis=-1):
    return jax.nn.softmax(x, axis=axis)
def _gelu(x):
    return jax.nn.gelu(x, approximate=True)
def _silu(x):
    return jax.nn.silu(x)
def _sigmoid(x):
    return jax.nn.sigmoid(x)
def _layernorm(x, axis=-1, eps=1e-5):
    m = jnp.mean(x, axis=axis, keepdims=True)
    v = jnp.var(x, axis=axis, keepdims=True)
    return (x - m) / jnp.sqrt(v + eps)
def _scatter_add(tgt, idx, src, axis=0):
    return tgt.at[idx].add(src)
def _segment_sum(src, seg, n):
    return jax.ops.segment_sum(src, seg, n)
class _Rng:
    def __init__(self, key):
        self._k = key
    def _next(self):
        self._k, sub = jax.random.split(self._k)
        return sub
    def normal(self, shape):
        return jax.random.normal(self._next(), shape, dtype=jnp.bfloat16)
    def randint(self, lo, hi, shape):
        return jax.random.randint(self._next(), shape, lo, hi, dtype=jnp.int32)
    def uniform(self, shape, lo=0.0, hi=1.0):
        return jax.random.uniform(self._next(), shape, jnp.bfloat16, lo, hi)
    def permutation(self, n):
        return jax.random.permutation(self._next(), n)


kernel_name = 'concat_heads__mha_block_cached__mha_block_cached__near_ridge'

def setup_inputs():
    _rng = _Rng(jax.random.key(int.from_bytes(__import__("os").urandom(4), "little")))
    _w = (lambda a: (lambda t: t.astype(jnp.bfloat16) if jnp.issubdtype(t.dtype, jnp.floating) else t)(jnp.asarray(a)))
    def _A_setup():
        B, Sq, D = 16, 80, 512
        H, Sk, Dh = 32, 80, 128
        return {
            "x": _w((lambda *s: _rng.normal(s) * 0.8)(B, Sq, D)),
            "k_cache": _w((lambda *s: _rng.normal(s) * 0.8)(B, H, Sk, Dh)),
            "v_cache": _w((lambda *s: _rng.normal(s) * 0.05)(B, H, Sk, Dh)),
            "wq": _w((lambda *s: _rng.normal(s) * 0.8)(D, H * Dh) * (D ** -0.5)),
            "wo": _w((lambda *s: _rng.normal(s) * 0.05)(H * Dh, D) * ((H * Dh) ** -0.5)),
        }
    _A_in = _A_setup()

    def _B_setup():
        B, Sq, D = 16, 80, 512
        H, Sk, Dh = 32, 80, 128
        return {
            "x": _w((lambda *s: _rng.normal(s) * 0.8)(B, Sq, D)),
            "k_cache": _w((lambda *s: _rng.normal(s) * 0.8)(B, H, Sk, Dh)),
            "v_cache": _w((lambda *s: _rng.normal(s) * 0.05)(B, H, Sk, Dh)),
            "wq": _w((lambda *s: _rng.normal(s) * 0.8)(D, H * Dh) * (D ** -0.5)),
            "wo": _w((lambda *s: _rng.normal(s) * 0.05)(H * Dh, D) * ((H * Dh) ** -0.5)),
        }
    _B_in = _B_setup()

    return {
        "A_x": _A_in["x"],
        "A_k_cache": _A_in["k_cache"],
        "A_v_cache": _A_in["v_cache"],
        "A_wq": _A_in["wq"],
        "A_wo": _A_in["wo"],
        "B_x": _B_in["x"],
        "B_k_cache": _B_in["k_cache"],
        "B_v_cache": _B_in["v_cache"],
        "B_wq": _B_in["wq"],
        "B_wo": _B_in["wo"],
    }

def reference(A_x, A_k_cache, A_v_cache, A_wq, A_wo, B_x, B_k_cache, B_v_cache, B_wq, B_wo):
    def _A_ref(x, k_cache, v_cache, wq, wo):
        B, Sq, D = x.shape
        H, Dh = 32, 128
        q = (lambda x, *d: x.transpose(*d))((x @ wq).reshape(B, Sq, H, Dh), 0, 2, 1, 3)
        scores = jnp.einsum("bhqd,bhkd->bhqk", q, k_cache) * (Dh ** -0.5)
        p = _softmax(scores, axis=-1)
        o = jnp.einsum("bhqk,bhkd->bhqd", p, v_cache)
        return (lambda x, *d: x.transpose(*d))(o, 0, 2, 1, 3).reshape(B, Sq, H * Dh) @ wo

    def _B_ref(x, k_cache, v_cache, wq, wo):
        B, Sq, D = x.shape
        H, Dh = 32, 128
        q = (lambda x, *d: x.transpose(*d))((x @ wq).reshape(B, Sq, H, Dh), 0, 2, 1, 3)
        scores = jnp.einsum("bhqd,bhkd->bhqk", q, k_cache) * (Dh ** -0.5)
        p = _softmax(scores, axis=-1)
        o = jnp.einsum("bhqk,bhkd->bhqd", p, v_cache)
        return (lambda x, *d: x.transpose(*d))(o, 0, 2, 1, 3).reshape(B, Sq, H * Dh) @ wo

    a = _A_ref(A_x, A_k_cache, A_v_cache, A_wq, A_wo)
    b = _B_ref(B_x, B_k_cache, B_v_cache, B_wq, B_wo)
    return jnp.concatenate([a, b], axis=-1)
```

```python
import math

import jax
import jax.numpy as jnp
from jax.experimental import pallas as pl
from jax.experimental.pallas import tpu as pltpu

B, SQ, D, H, SK, DH = 16, 80, 512, 32, 80, 128
M = B * SQ
G, UB = 4, 4
NG, NU = H // G, B // UB
NS = 2 * NG
W, RU = G * DH, UB * SQ
LQ, LO = 2, 1
PQ, PO = 7 ** LQ, 7 ** LO
SCALE = DH ** -0.5 * math.log2(math.e)
LEAD = 3
SLOTS = 2 * UB * G + UB // 2 * PO * 2
ORDER = (3, 5, 7, 1, 4, 2, 6)
f32, bf16, u32 = jnp.float32, jnp.bfloat16, jnp.uint32

SEQ_FIRST = "|XXXXX|W.qqqqqq|XXXXXqqqq|XXXqqXXqq|ssqXqXsqsXqpXpsqsXppssqqpppqp|VssqqssVqppVsqVpVspssqpqVpVpp|Vssossppsosoop|wwwwwoosoppsopwppww"
SEQ_SECOND = "|sqoVVosoqssqqqsVppqoVspsqVspqppqoppo|swsqVqswqsoVpsqssosqpVwqwqspppwosppospwqpwsqqwqsqpssoppqsoop|vpsqsvpqsvqsppvpovssqqspspppoqpvpovv"
SEQ_LOOP = "osqsqqosqsowqpspqpossqpsqpowpqpposswqsqqsssppqpopqossqqpvsvvpopsowspqpvqsvvqovsqwppssvvpoqpqspqoswspqsvqspvqppwovvsswpqsspqpopppvvov"
SEQ_LAST = "!sosssspoppsssopo!pppopooo!"
STARTUP = "x0|q0|x1|x2|x3 k00|k01 o0|k02|q1|k03 o1|k10 k11 q2|o2 k12|k13 k20 k21 k22 q3 o3"


def _halves(w):
    return [pltpu.unpack_elementwise(w, index=i, packed_dtype=bf16, unpacked_dtype=f32) for i in range(2)]


def _pack(lo, hi):
    return pltpu.pack_elementwise([lo, hi], packed_dtype=bf16)


def _pack_rows(v):
    groups = range(v.shape[0] // 16)
    return _pack(*[jnp.concatenate([v[16 * z + 8 * i:16 * z + 8 * i + 8] for z in groups], axis=0) for i in range(2)])


def _bf16(w):
    return pltpu.bitcast(w, bf16)


def _words(v):
    return pltpu.bitcast(v, u32)


def _quadrants(b, level):
    h = 2 ** (level - 1)
    return [{(r, c): b[R * h + r, C * h + c] for r in range(h) for c in range(h)} for R in range(2) for C in range(2)]


def _add(x, y):
    return {k: x[k] + y[k] for k in x}


def _sub(x, y):
    return {k: x[k] - y[k] for k in x}


def _left_operands(b, level):
    if level == 0:
        yield b[0, 0]
        return
    a11, a12, a21, a22 = _quadrants(b, level)
    make = {1: lambda: _add(a11, a22), 2: lambda: _add(a21, a22), 3: lambda: a11, 4: lambda: a22,
            5: lambda: _add(a11, a12), 6: lambda: _sub(a21, a11), 7: lambda: _sub(a12, a22)}
    for i in ORDER:
        yield from _left_operands(make[i](), level - 1)


def _right_operands(b, level):
    if level == 0:
        yield b[0, 0]
        return
    b11, b12, b21, b22 = _quadrants(b, level)
    make = {1: lambda: _add(b11, b22), 2: lambda: b11, 3: lambda: _sub(b12, b22), 4: lambda: _sub(b21, b11),
            5: lambda: b22, 6: lambda: _add(b11, b12), 7: lambda: _add(b21, b22)}
    for i in ORDER:
        yield from _right_operands(make[i](), level - 1)


def _plain_right(level):
    if level == 0:
        return [0]
    outer = [{2: 0, 5: 1}.get(i) for i in ORDER]
    return [None if R is None or b is None else R * 2 ** (level - 1) + b for R in outer for b in _plain_right(level - 1)]


def _combine(product, level, emit, base=0, store=None):
    if level == 0:
        emit((0, 0), product(base))
        yield
        return
    h = 2 ** (level - 1)
    m3, m4, m5, t11, t22 = [store(i) if store else {} for i in range(5)]

    def out(R, C, k, v):
        emit((R * h + k[0], C * h + k[1]), v)

    def on3(k, v):
        m3[k] = v

    def on5(k, v):
        m5[k] = v
        out(0, 1, k, m3[k] + v)

    def on7(k, v):
        t11[k] = v - m5[k]

    def on1(k, v):
        t11[k] = t11[k] + v
        t22[k] = m3[k] + v

    def on4(k, v):
        m4[k] = v
        out(0, 0, k, t11[k] + v)

    def on2(k, v):
        out(1, 0, k, v + m4[k])
        t22[k] = t22[k] - v

    def on6(k, v):
        out(1, 1, k, t22[k] + v)

    for j, on in enumerate((on3, on5, on7, on1, on4, on2, on6)):
        yield from _combine(product, level - 1, on, base + j * 7 ** (level - 1))


def _interleave(jobs):
    ticks = sorted(((i + 0.5) / n, j) for j, (_, n) in enumerate(jobs) for i in range(n))
    for _, j in ticks:
        next(jobs[j][0])


def _branch(cond, fn):
    def once(_, carry):
        fn()
        return carry
    jax.lax.fori_loop(0, cond.astype(jnp.int32), once, 0)


def _kernel(ax, ak, av, awq, awo, bx, bk, bv, bwq, bwo, out, xb, kb, vb, wqb, wob, xs, wqs, wos, tmp, part, acc, ob, sem):
    def cols(g):
        return pl.ds(g * W if isinstance(g, int) else pl.multiple_of(g * W, W), W)

    def cp_wq(br, g, n):
        return pltpu.make_async_copy((awq, bwq)[br].at[:, cols(g)], wqb.at[br * NG + g], sem.at[n])

    def cp_wo(br, g, n):
        return pltpu.make_async_copy((awo, bwo)[br].at[cols(g)], wob.at[br * NG + g], sem.at[n])

    def cp_kv(br, g, n, u=None):
        rows = pl.ds(0, B) if u is None else pl.ds(u * UB, UB)
        return [pltpu.make_async_copy(src[br].at[rows, pl.ds(g * G, G)], dst.at[br * NG + g, rows], sem.at[n])
                for src, dst in (((ak, bk), kb), ((av, bv), vb))]

    def cp_x(br, n, u=None):
        rows = pl.ds(0, M) if u is None else pl.ds(u * RU, RU)
        return pltpu.make_async_copy((ax, bx)[br].at[rows], xb.at[br, rows], sem.at[n])

    def cp_out(br, u=None):
        rows = pl.ds(0, M) if u is None else pl.ds(u * RU, RU)
        return pltpu.make_async_copy(ob.at[br, rows], out.at[rows, pl.ds(br * D, D)], sem.at[LEAD + 1])

    def convert(br, r0, r1):
        for c in range(D // 128):
            ob[br, r0:r1, c * 128:(c + 1) * 128] = _bf16(_pack_rows(acc[br, c, r0:r1, :]))

    def prep_x(br, units):
        for u in units:
            for p in range(SQ // 16):
                hv = {(r, c): [h * SCALE for h in _halves(_words(xb[br, pl.ds((u * UB + r) * SQ + p * 16, 16), c * 128:(c + 1) * 128]))]
                      for r in range(4) for c in range(4)}
                for i, ops in enumerate(zip(*[_left_operands({k: v[z] for k, v in hv.items()}, LQ) for z in range(2)])):
                    xs[i, pl.ds((u * SQ + p * 16) // 2, 8), :] = _pack(*ops)
                yield

    def prep_w(src, s, dst, bank, level):
        n = 2 ** level
        kk, nn = src.shape[1] // n, src.shape[2] // n
        for cc in range(nn // 128):
            for p in range(kk // 16):
                hv = {(r, c): _halves(_words(src[s, pl.ds(r * kk + p * 16, 16), pl.ds(c * nn + cc * 128, 128)]))
                      for r in range(n) for c in range(n)}
                for i, ops in enumerate(zip(*[_right_operands({k: v[z] for k, v in hv.items()}, level) for z in range(2)])):
                    if _plain_right(level)[i] is None:
                        dst[bank, i, cc, p * 8:(p + 1) * 8, :] = _pack(*ops)
                yield

    def weight(src, s, dst, level, i, cc):
        b = _plain_right(level)[i]
        if b is None:
            return _bf16(dst[s % 2, i, cc])
        kk, nn = src.shape[1] // 2 ** level, src.shape[2] // 2 ** level
        return src[s, b * kk:(b + 1) * kk, b * nn + cc * 128:b * nn + (cc + 1) * 128]

    groups = [g.split() for g in STARTUP.split("|")]
    state = {"started": 0, "waited": 0, "have": []}

    def group(n):
        res, z = [], n % (LEAD + 1)
        for name in groups[n]:
            i = int(name[1])
            res += {"x": lambda: [cp_x(0, z, i)], "q": lambda: [cp_wq(0, i, z)], "o": lambda: [cp_wo(0, i, z)],
                    "k": lambda: cp_kv(0, i, z, int(name[-1]))}[name[0]]()
        return res

    def start_groups(upto):
        for n in range(state["started"], min(upto, len(groups))):
            for c in group(n):
                c.start()
            state["started"] = n + 1

    def stage():
        for c in group(state["waited"]):
            c.wait()
        state["have"] += groups[state["waited"]]
        state["waited"] += 1
        start_groups(state["waited"] + LEAD)

    def body(s, seq):
        peeled = isinstance(s, int)
        early = peeled and s < 2
        pin = 0 if peeled else s // (2 * NS)

        def need(name):
            assert not early or name in state["have"], name

        def where(u):
            return (s, u) if u >= 0 else (s - 1, u + NU)

        def slot(kind, u, k):
            return (u % NU) * SLOTS + kind * UB * G + k

        def units(first):
            return [u for u in range(first, first + NU) if not (peeled and (u < 0 if s == 0 else s == NS and u >= 0))]

        class Partial:
            def __init__(self, i):
                self.i = i

            def __setitem__(self, k, v):
                part[pin, self.i, 2 * k[0] + k[1]] = v

            def __getitem__(self, k):
                return part[pin, self.i, 2 * k[0] + k[1]]

        def q_stream():
            for u in units(0):
                def emit(rc, v):
                    tmp[pin, slot(0, u, rc[0] * G + rc[1])] = _pack_rows(v)

                def product(i):
                    a = _bf16(xs[i, u * SQ // 2:(u + 1) * SQ // 2, :])
                    return jnp.dot(a, weight(wqb, s, wqs, LQ, i, 0), preferred_element_type=f32)
                yield from _combine(product, LQ, emit, store=Partial)

        heads = [(2 * t + r, 2 * c + kt) for t in range(UB // 2) for kt in range(2) for r, c in ((0, 0), (1, 1), (0, 1), (1, 0))]

        def s_stream():
            for u in units(-1):
                ss, uu = where(u)
                for j, h in heads:
                    need(f"k{ss}{uu}" if early else None)
                    sc = jax.lax.dot_general(_bf16(tmp[pin, slot(0, u, j * G + h)]), kb[ss, uu * UB + j, h],
                                             (((1,), (1,)), ((), ())), preferred_element_type=f32)
                    sc = jnp.concatenate([sc, jnp.full((SQ, 128 - SK), -jnp.inf, f32)], axis=1)
                    e = jnp.exp2(sc - jnp.max(sc, axis=-1, keepdims=True))
                    r = pl.reciprocal(jnp.sum(e, axis=-1, keepdims=True), approx=True)
                    tmp[pin, slot(1, u, j * G + h)] = _pack_rows(e * r)
                    yield

        def p_stream():
            for u in units(-1):
                ss, uu = where(u)
                blk = {}
                for j, h in heads:
                    p = _bf16(tmp[pin, slot(1, u, j * G + h)])[:, :SK]
                    v = jnp.dot(p, vb[ss, uu * UB + j, h], preferred_element_type=f32)
                    blk[j % 2, h // 2] = v
                    ops = {(0, 0): {3: lambda: v}, (1, 1): {4: lambda: v, 1: lambda: blk[0, 0] + v},
                           (0, 1): {5: lambda: blk[0, 0] + v, 7: lambda: v - blk[1, 1]},
                           (1, 0): {2: lambda: v + blk[1, 1], 6: lambda: v - blk[0, 0]}}[j % 2, h // 2]
                    for i, op in ops.items():
                        tmp[pin, slot(2, u, (j // 2 * PO + ORDER.index(i)) * 2 + h % 2)] = _pack_rows(op())
                    yield

        def o_stream():
            for u in units(-2):
                ss, uu = where(u)
                for t in range(UB // 2):
                    for cc in range(2):
                        def emit(rc, v):
                            r0, cb = (uu * UB + 2 * t + rc[0]) * SQ, rc[1] * 2 + cc
                            if not (peeled and s == 0):
                                v = acc[ss // NG, cb, r0:r0 + SQ, :] + v
                            if peeled and s == NS:
                                ob[1, r0:r0 + SQ, cb * 128:(cb + 1) * 128] = _bf16(_pack_rows(v))
                            else:
                                acc[ss // NG, cb, r0:r0 + SQ, :] = v

                        def product(i):
                            a = jnp.concatenate([_bf16(tmp[pin, slot(2, u, (t * PO + i) * 2 + kt)]) for kt in range(2)], axis=1)
                            return jnp.dot(a, weight(wob, ss, wos, LO, i, cc), preferred_element_type=f32)
                        yield from _combine(product, LO, emit)

        nxt = s + 1 if peeled else jnp.minimum(s + 1, NS - 1)
        streams = {"q": (q_stream(), PQ * len(units(0))), "s": (s_stream(), UB * G * len(units(-1))),
                   "p": (p_stream(), UB * G * len(units(-1))), "o": (o_stream(), 4 * PO * len(units(-2))),
                   "w": (prep_w(wqb, nxt, wqs, (s + 1) % 2, LQ), 8), "v": (prep_w(wob, nxt, wos, (s + 1) % 2, LO), 32),
                   "W": (prep_w(wqb, s, wqs, s % 2, LQ), 8), "V": (prep_w(wob, s, wos, s % 2, LO), 32),
                   "X": (prep_x(0, range(NU)), NU * SQ // 16)}
        pending, done, sent = [], dict.fromkeys(streams, 0), 0
        for tok in seq + ".":
            if tok in streams:
                gen, total = streams[tok]
                assert total % seq.count(tok) == 0
                pending.append((gen, total // seq.count(tok)))
                done[tok] += total // seq.count(tok)
                if early and tok in "wvWVX":
                    need({"w": f"q{s + 1}", "v": f"o{s + 1}", "W": f"q{s}", "V": f"o{s}", "X": f"x{(done[tok] - 1) // 5}"}[tok])
            if tok not in "wvWVX":
                _interleave(pending)
                pending = []
            if tok == "|":
                stage()
            if tok == "!":
                for u in range(sent, NU - 2 + done["o"] // (4 * PO)):
                    cp_out(1, u).start()
                    sent = u + 1
        assert all(done[k] == streams[k][1] for k in "qspo")

    start_groups(2)
    for c in range(D // 128):
        acc[0, c, (NU - 2) * RU:, :] = jnp.zeros((2 * RU, 128), f32)
        acc[1, c] = jnp.zeros((M, 128), f32)
    body(0, SEQ_FIRST)
    body(1, SEQ_SECOND)
    while state["waited"] < len(groups):
        stage()

    def step_copies(kv, w):
        return cp_kv(*kv, 0) + ([cp_wq(*w, 0), cp_wo(*w, 0)] if w else [])

    def launch(copies):
        for c in copies:
            c.start()

    def step(s, carry):
        @pl.when(s > 2)
        def _():
            for c in step_copies((0, 0), None):
                c.wait()

        @pl.when(jnp.logical_and(s > 2, s + 1 < NS))
        def _():
            cp_wq(0, 0, 0).wait()
            cp_wo(0, 0, 0).wait()

        def rare_events():
            @pl.when(s == 3)
            def _():
                for c in cp_kv(0, 2, 0, NU - 1):
                    c.wait()
            _branch(s == 2, lambda: launch(cp_kv(0, 2, 0, NU - 1)))
            pl.when(s == NG - 1)(lambda: cp_x(1, 0).wait())
            _branch(s == NG - 2, lambda: launch(step_copies((0, NG - 1), (1, 0)) + [cp_x(1, 0)]))
            _branch(s == NG, lambda: list(prep_x(1, range(NU))))
            _branch(s == NG + 1, lambda: (convert(0, 0, M), cp_out(0).start()))
            _branch(s == NS - 2, lambda: launch(step_copies((1, NG - 1), None)))
        _branch(jnp.logical_or(s <= NG + 1, s == NS - 2), rare_events)
        _branch(s + 2 < NG, lambda: launch(step_copies((0, s + 1), (0, s + 2))))
        _branch(jnp.logical_and(s + 1 >= NG, s + 2 < NS), lambda: launch(step_copies((1, s + 1 - NG), (1, s + 2 - NG))))
        body(s, SEQ_LOOP)
        return carry
    jax.lax.fori_loop(2, NS, step, 0)
    convert(1, 0, (NU - 2) * RU)
    body(NS, SEQ_LAST)
    cp_out(0).wait()
    for u in range(NU):
        cp_out(1, u).wait()


@jax.jit
def pallas_concat_heads__mha_block_cached__mha_block_cached__near_ridge_kernel(
        A_x, A_k_cache, A_v_cache, A_wq, A_wo, B_x, B_k_cache, B_v_cache, B_wq, B_wo):
    vmem = pltpu.VMEM
    out = pl.pallas_call(
        _kernel,
        out_shape=jax.ShapeDtypeStruct((M, 2 * D), bf16),
        in_specs=[pl.BlockSpec(memory_space=pl.ANY)] * 10,
        out_specs=pl.BlockSpec(memory_space=pl.ANY),
        scratch_shapes=[
            vmem((2, M, D), bf16),
            vmem((NS, B, G, SK, DH), bf16),
            vmem((NS, B, G, SK, DH), bf16),
            vmem((NS, D, W), bf16),
            vmem((NS, W, D), bf16),
            vmem((PQ, NU * SQ // 2, 128), u32),
            vmem((2, PQ, 1, D // 8, 128), u32),
            vmem((2, PO, 2, W // 4, 128), u32),
            vmem((2, NU * SLOTS, SQ // 2, 128), u32),
            vmem((2, 5, 4, SQ, 128), f32),
            vmem((2, D // 128, M, 128), f32),
            vmem((2, M, D), bf16),
            pltpu.SemaphoreType.DMA((LEAD + 2,)),
        ],
        compiler_params=pltpu.CompilerParams(vmem_limit_bytes=120 * 2 ** 20, disable_bounds_checks=True),
    )(A_x.reshape(M, D), A_k_cache, A_v_cache, A_wq, A_wo, B_x.reshape(M, D), B_k_cache, B_v_cache, B_wq, B_wo)
    return out.reshape(B, SQ, 2 * D)
```
